```python
import jax
import jax.numpy as jnp

def _softmax(x, axis=-1):
    return jax.nn.softmax(x, axis=axis)
def _gelu(x):
    return jax.nn.gelu(x, approximate=True)
def _silu(x):
    return jax.nn.silu(x)
def _sigmoid(x):
    return jax.nn.sigmoid(x)
def _layernorm(x, axis=-1, eps=1e-5):
    m = jnp.mean(x, axis=axis, keepdims=True)
    v = jnp.var(x, axis=axis, keepdims=True)
    return (x - m) / jnp.sqrt(v + eps)
def _scatter_add(tgt, idx, src, axis=0):
    return tgt.at[idx].add(src)
def _segment_sum(src, seg, n):
    return jax.ops.segment_sum(src, seg, n)
class _Rng:
    def __init__(self, key):
        self._k = key
    def _next(self):
        self._k, sub = jax.random.split(self._k)
        return sub
    def normal(self, shape):
        return jax.random.normal(self._next(), shape, dtype=jnp.bfloat16)
    def randint(self, lo, hi, shape):
        return jax.random.randint(self._next(), shape, lo, hi, dtype=jnp.int32)
    def uniform(self, shape, lo=0.0, hi=1.0):
        return jax.random.uniform(self._next(), shape, jnp.bfloat16, lo, hi)
    def permutation(self, n):
        return jax.random.permutation(self._next(), n)


kernel_name = 'gated_mix__sliding_block_cached__mixer_s_mlp__decode'

def setup_inputs():
    _rng = _Rng(jax.random.key(int.from_bytes(__import__("os").urandom(4), "little")))
    _w = (lambda a: (lambda t: t.astype(jnp.bfloat16) if jnp.issubdtype(t.dtype, jnp.floating) else t)(jnp.asarray(a)))
    def _A_setup():
        B, Sq, D = 1, 1, 576
        Hq, Hkv, Sk, Dh = 32, 16, 65536, 128
        assert Hq % Hkv == 0, (Hq, Hkv)
        return {
            "x": _w((lambda *s: _rng.normal(s) * 0.05)(B, Sq, D)),
            "k_cache": _w((lambda *s: _rng.normal(s) * 0.05)(B, Hkv, Sk, Dh)),
            "v_cache": _w((lambda *s: _rng.normal(s) * 0.05)(B, Hkv, Sk, Dh)),
            "wq": _w((lambda *s: _rng.normal(s) * 0.05)(D, Hq * Dh) * (D ** -0.5)),
            "wo": _w((lambda *s: _rng.normal(s) * 0.05)(Hq * Dh, D) * ((Hq * Dh) ** -0.5)),
        }
    _A_in = _A_setup()

    def _B_setup():
        B, S, D, F = 1, 1, 576, 4608
        return {
            "x":  _w((lambda *s: _rng.normal(s) * 0.05)(B, S, D)),
            "w1": _w((lambda *s: _rng.normal(s) * 0.05)(D, D) * (D ** -0.5)),
            "w2": _w((lambda *s: _rng.normal(s) * 0.05)(D, D) * (D ** -0.5)),
            "w3": _w((lambda *s: _rng.normal(s) * 0.05)(D, F) * (D ** -0.5)),
            "w4": _w((lambda *s: _rng.normal(s) * 0.05)(F, D) * (F ** -0.5)),
        }
    _B_in = _B_setup()

    return {
        "A_x": _A_in["x"],
        "A_k_cache": _A_in["k_cache"],
        "A_v_cache": _A_in["v_cache"],
        "A_wq": _A_in["wq"],
        "A_wo": _A_in["wo"],
        "B_x": _B_in["x"],
        "B_w1": _B_in["w1"],
        "B_w2": _B_in["w2"],
        "B_w3": _B_in["w3"],
        "B_w4": _B_in["w4"],
        "gate_w": _w((lambda *s: _rng.normal(s) * 0.05)(576)),
    }

def reference(A_x, A_k_cache, A_v_cache, A_wq, A_wo, B_x, B_w1, B_w2, B_w3, B_w4, gate_w):
    def _A_ref(x, k_cache, v_cache, wq, wo):
        B, Sq, D = x.shape
        Hq, Dh = 32, 128
        Hkv, Sk = k_cache.shape[1], k_cache.shape[2]
        W = min(4096, max(256, Sk // 4))
        rep = Hq // Hkv
        q = (lambda x, *d: x.transpose(*d))((x @ wq).reshape(B, Sq, Hq, Dh), 0, 2, 1, 3)
        k = jnp.repeat(k_cache[:, :, Sk - W:, :], rep, axis=1)
        v = jnp.repeat(v_cache[:, :, Sk - W:, :], rep, axis=1)
        scores = jnp.einsum("bhqd,bhkd->bhqk", q, k) * (Dh ** -0.5)
        p = _softmax(scores, axis=-1)
        o = jnp.einsum("bhqk,bhkd->bhqd", p, v)
        return (lambda x, *d: x.transpose(*d))(o, 0, 2, 1, 3).reshape(B, Sq, Hq * Dh) @ wo

    def _B_ref(x, w1, w2, w3, w4):
        B, S, D = x.shape
        h = _gelu(_layernorm(x, axis=-1) @ w1)
        c = D // 4
        g0 = jnp.pad(h[:, :, 0*c:1*c], ((0, 0), (1, 0), (0, 0)))[:, :S, :]
        g1 = jnp.pad(h[:, :, 1*c:2*c], ((0, 0), (0, 1), (0, 0)))[:, 1:, :]
        g2 = jnp.pad(h[:, :, 2*c:3*c], ((0, 0), (2, 0), (0, 0)))[:, :S, :]
        g3 = jnp.pad(h[:, :, 3*c:   ], ((0, 0), (0, 2), (0, 0)))[:, 2:, :]
        hs = jnp.concatenate([g0, g1, g2, g3], axis=-1) @ w2
        x1 = x + hs
        h2 = _gelu(_layernorm(x1, axis=-1) @ w3) @ w4
        return x1 + h2

    x = A_x
    g = _sigmoid((x * gate_w).sum(-1, keepdims=True))
    a = _A_ref(x, A_k_cache, A_v_cache, A_wq, A_wo)
    b = _B_ref(x, B_w1, B_w2, B_w3, B_w4)
    return g * a + (1 - g) * b
```

```python
import jax
import jax.numpy as jnp
from jax import lax
from jax.experimental import pallas as pl
from jax.experimental.pallas import tpu as pltpu

F32, BF16 = jnp.float32, jnp.bfloat16
NT = (((1,), (1,)), ((), ()))
HQ, DH = 32, 128
ROWS = 8
KV_PIECE_ROWS = 128
W_PIECE_ROWS = 8
W_UNIT_ROWS = 144
W4_BOUNDS = (0, 128, 256, 384, 512, 576)
AHEAD = 128
NSEM = 4


def _interleave(streams):
    return [p for group in zip(*streams) for p in group]


def _weight_pieces(name, r0, r1, ncols):
    half = ncols // 2
    pieces = [
        (name, r, c, half)
        for r in range(r0, r1, W_PIECE_ROWS)
        for c in (0, half)
    ]
    n = len(pieces) // 4
    return _interleave([pieces[i * n:(i + 1) * n] for i in range(4)])


def _plan(d, ff, hkv, window):
    units = []

    def weight(name, ncols, bounds):
        for r0, r1 in zip(bounds[:-1], bounds[1:]):
            units.append((name, (r0, r1), _weight_pieces(name, r0, r1, ncols)))

    even = tuple(range(0, d + 1, W_UNIT_ROWS))
    weight("wq", HQ * DH, even)
    weight("w3", ff, even)
    for h in range(hkv):
        k = [("k", h, r) for r in range(0, window, KV_PIECE_ROWS)]
        v = [("v", h, r) for r in range(0, window, KV_PIECE_ROWS)]
        n = len(k) // 2
        units.append(("kv", h, _interleave([k[:n], v[:n], k[n:], v[n:]])))
    weight("wo", HQ * DH, even)
    weight("w4", ff, W4_BOUNDS)
    return units


@jax.jit
def pallas_gated_mix__sliding_block_cached__mixer_s_mlp__decode_kernel(
    A_x: jax.Array,
    A_k_cache: jax.Array,
    A_v_cache: jax.Array,
    A_wq: jax.Array,
    A_wo: jax.Array,
    B_x: jax.Array,
    B_w1: jax.Array,
    B_w2: jax.Array,
    B_w3: jax.Array,
    B_w4: jax.Array,
    gate_w: jax.Array,
):
    del B_x, B_w1, B_w2
    d = A_x.shape[-1]
    ff = B_w3.shape[-1]
    hkv, sk = A_k_cache.shape[1], A_k_cache.shape[2]
    assert A_x.shape == (1, 1, d) and HQ == 2 * hkv
    window = min(4096, max(256, sk // 4))
    start = sk - window
    units = _plan(d, ff, hkv, window)

    def kernel(x_hbm, k_hbm, v_hbm, wq_hbm, wo_hbm, w3_hbm, w4_hbm, g_hbm, o_ref,
               xb, gb, kb, vb, wqb, wob, w3b, w4b, qs, outs, sems, small_sem):
        weights = dict(wq=(wq_hbm, wqb), wo=(wo_hbm, wob), w3=(w3_hbm, w3b), w4=(w4_hbm, w4b))
        caches = dict(k=(k_hbm, kb), v=(v_hbm, vb))
        pieces = [(u, p) for u, (_, _, ps) in enumerate(units) for p in ps]
        progress = dict(issued=0, waited=0)

        def issue_until(limit):
            while progress["issued"] < min(limit, len(pieces)):
                u, p = pieces[progress["issued"]]
                if u >= progress["waited"] + NSEM:
                    break
                if p[0] in caches:
                    src, dst = caches[p[0]]
                    src = src.at[0, p[1], pl.ds(start + p[2], KV_PIECE_ROWS), :]
                    dst = dst.at[p[1], pl.ds(p[2], KV_PIECE_ROWS), :]
                else:
                    block = (pl.ds(p[1], W_PIECE_ROWS), pl.ds(p[2], p[3]))
                    src, dst = (r.at[block] for r in weights[p[0]])
                pltpu.make_async_copy(src, dst, sems.at[u % NSEM]).start(
                    priority=progress["issued"] % 2)
                progress["issued"] += 1

        def wait_unit(u):
            kind, arg, _ = units[u]
            if kind == "kv":
                filled = (kb.at[arg], vb.at[arg])
            else:
                filled = (weights[kind][1].at[pl.ds(arg[0], arg[1] - arg[0]), :],)
            for r in filled:
                pltpu.make_async_copy(r, r, sems.at[u % NSEM]).wait()
            progress["waited"] = u + 1

        issue_until(4)
        small = (pltpu.make_async_copy(x_hbm, xb, small_sem),
                 pltpu.make_async_copy(g_hbm, gb, small_sem))
        for c in small:
            c.start()
        issue_until(AHEAD)
        for c in small:
            c.wait()

        x = xb[0].astype(F32)
        gate = jax.nn.sigmoid(
            jnp.sum(x * gb[...].astype(F32).reshape(1, d), axis=-1, keepdims=True))
        centered = x - jnp.mean(x, axis=-1, keepdims=True)
        var = jnp.mean(centered * centered, axis=-1, keepdims=True)
        xn = jnp.broadcast_to(centered / jnp.sqrt(var + 1e-5), (ROWS, d)).astype(BF16)
        odd = lax.broadcasted_iota(jnp.int32, (ROWS, DH), 0) % 2 == 1

        issued_goal = AHEAD
        for u, (kind, arg, ps) in enumerate(units):
            wait_unit(u)
            issued_goal += len(ps)
            issue_until(issued_goal)
            if kind == "wq" and arg[1] == d:
                x8 = jnp.broadcast_to(x, (ROWS, d)).astype(BF16)
                q = jnp.dot(x8, wqb[...], preferred_element_type=F32)
                for h in range(hkv):
                    c = 2 * DH * h
                    qs[h] = jnp.where(odd, q[:, c + DH:c + 2 * DH], q[:, c:c + DH]).astype(BF16)
            elif kind == "w3" and arg[1] == d:
                hidden = jnp.dot(xn, w3b[...], preferred_element_type=F32)
                hidden = jax.nn.gelu(hidden, approximate=True).astype(BF16)
            elif kind == "kv":
                s = lax.dot_general(qs[arg], kb[arg], NT, preferred_element_type=F32)
                s = s * (DH ** -0.5)
                p = jnp.exp(s - jnp.max(s, axis=-1, keepdims=True))
                denom = jnp.sum(p, axis=-1, keepdims=True)
                outs[arg] = jnp.dot(p.astype(BF16), vb[arg], preferred_element_type=F32) / denom
            elif kind == "wo" and arg[1] == d:
                cols = []
                for h in range(hkv):
                    o = outs[h]
                    cols += [jnp.broadcast_to(o[i:i + 1], (ROWS, DH)) for i in range(2)]
                merged = jnp.concatenate(cols, axis=1).astype(BF16)
                attn = lax.dot_general(merged, wob[...], NT, preferred_element_type=F32)[0:1]
                base = gate * attn + (1.0 - gate) * x
            elif kind == "w4":
                r0, r1 = arg
                mlp = lax.dot_general(hidden, w4b[pl.ds(r0, r1 - r0), :], NT,
                                      preferred_element_type=F32)[0:1]
                o_ref[0, :, pl.ds(r0, r1 - r0)] = (
                    base[:, r0:r1] + (1.0 - gate) * mlp).astype(BF16)

    hbm = pl.BlockSpec(memory_space=pl.ANY)
    return pl.pallas_call(
        kernel,
        name="gated_mix_decode",
        out_shape=jax.ShapeDtypeStruct((1, 1, d), BF16),
        in_specs=[hbm] * 8,
        out_specs=pl.BlockSpec(memory_space=pltpu.VMEM),
        scratch_shapes=[
            pltpu.VMEM((1, 1, d), BF16),
            pltpu.VMEM((d,), BF16),
            pltpu.VMEM((hkv, window, DH), BF16),
            pltpu.VMEM((hkv, window, DH), BF16),
            pltpu.VMEM((d, HQ * DH), BF16),
            pltpu.VMEM((d, HQ * DH), BF16),
            pltpu.VMEM((d, ff), BF16),
            pltpu.VMEM((d, ff), BF16),
            pltpu.VMEM((hkv, ROWS, DH), BF16),
            pltpu.VMEM((hkv, ROWS, DH), F32),
            pltpu.SemaphoreType.DMA((NSEM,)),
            pltpu.SemaphoreType.DMA(()),
        ],
        compiler_params=pltpu.CompilerParams(vmem_limit_bytes=100 * 1024 * 1024),
    )(A_x, A_k_cache, A_v_cache, A_wq, A_wo.T, B_w3, B_w4.T, gate_w)
```

```python
import jax
import jax.numpy as jnp
from jax import lax
from jax.experimental import pallas as pl
from jax.experimental.pallas import tpu as pltpu

F32, BF16 = jnp.float32, jnp.bfloat16
CONTRACT_LAST = (((1,), (1,)), ((), ()))
HQ, DH = 32, 128
LANES = 128
ROWS = 8

KV_PIECE_ROWS = 128
WEIGHT_PIECE_ROWS = 8
HEADS_PER_UNIT = 4
TAIL_COLS = (2560, 1024, 1024)
NUM_SEMS = 5
IN_FLIGHT = 104
TICK = 32
LAG = 20


def _round_robin(streams):
    longest = max(len(s) for s in streams)
    return [s[i] for i in range(longest) for s in streams if i < len(s)]


def _streams(pieces, count):
    cuts = [len(pieces) * i // count for i in range(count + 1)]
    return [pieces[a:b] for a, b in zip(cuts[:-1], cuts[1:])]


def _blocks(name, r0, r1, c0, c1, rows, cols):
    return [(name, r, rows, c, cols)
            for r in range(r0, r1, rows) for c in range(c0, c1, cols)]


def _plan_units(d, ff, hkv, window):
    def weight(name, ncols, r0, r1):
        return _blocks(name, r0, r1, 0, ncols, WEIGHT_PIECE_ROWS, ncols // 2)

    units = [(
        _round_robin(_streams(weight("wq", HQ * DH, 0, d), 4)
                     + _streams(weight("w3", ff, 0, d), 4)),
        [("pre",), ("query",), ("hidden",)],
    )]
    for first in range(0, hkv, HEADS_PER_UNIT):
        heads = range(first, first + HEADS_PER_UNIT)
        units.append((
            _round_robin([[(t, h, r) for r in range(0, window, KV_PIECE_ROWS)]
                          for h in heads for t in ("k", "v")]),
            [("head", h) for h in heads],
        ))
    units.append((_round_robin(_streams(weight("wo", HQ * DH, 0, d), 8)), [("project",)]))

    whole = d // LANES * LANES
    last = whole - LANES
    for row_ranges in (((whole, d), (0, last - LANES)), ((last - LANES, last),)):
        pieces = [p for r0, r1 in row_ranges for p in weight("w4", ff, r0, r1)]
        stages = [("down", r, min(r + LANES, r1), 0, ff)
                  for r0, r1 in row_ranges for r in range(r0, r1, LANES)]
        units.append((_round_robin(_streams(pieces, 4)), stages))
    c0 = 0
    for cols in TAIL_COLS:
        rows, width = (WEIGHT_PIECE_ROWS, cols // 2) if cols > 2048 else (16384 // cols, cols)
        pieces = _blocks("w4", last, whole, c0, c0 + cols, rows, width)
        units.append((_round_robin(_streams(pieces, 4)), [("down", last, whole, c0, c0 + cols)]))
        c0 += cols
    assert c0 == ff
    return units


def _plan_program(units):
    pieces = [(u, p) for u, (ps, _) in enumerate(units) for p in ps]
    n = len(pieces)
    lag = LAG + (n - LAG) % 2
    copies = [(u, p, i % 2 if i < n - lag else 1) for i, (u, p) in enumerate(pieces)]
    queues = [[i for i in range(n) if copies[i][2] == q] for q in (0, 1)]
    pairs = zip(queues[0], queues[1][lag:])
    order = queues[1][:lag] + [i for pair in pairs for i in pair]
    assert sorted(order) == list(range(n))

    steps, ready, started = [], [], set()
    waited = done = end = 0

    def top_up():
        while len(started) < min(waited + IN_FLIGHT, n):
            i = order[len(started)]
            if copies[i][0] >= done + NUM_SEMS:
                break
            steps.append(("start", i))
            started.add(i)

    top_up()
    for ps, stages in units:
        end += len(ps)
        while waited < end:
            stop = end if end - waited < TICK * 3 // 2 else waited + TICK
            assert started.issuperset(range(waited, stop))
            steps += [("wait", i) for i in range(waited, stop)]
            waited = stop
            if waited == end:
                done += 1
                ready += stages
            top_up()
            count = len(ready) if len(started) == n else 1
            steps += [("run", s) for s in ready[:count]]
            ready = ready[count:]
    assert not ready
    return copies, steps


@jax.jit
def pallas_gated_mix__sliding_block_cached__mixer_s_mlp__decode_kernel(
    A_x: jax.Array,
    A_k_cache: jax.Array,
    A_v_cache: jax.Array,
    A_wq: jax.Array,
    A_wo: jax.Array,
    B_x: jax.Array,
    B_w1: jax.Array,
    B_w2: jax.Array,
    B_w3: jax.Array,
    B_w4: jax.Array,
    gate_w: jax.Array,
):
    del B_x, B_w1, B_w2
    d = A_x.shape[-1]
    ff = B_w3.shape[-1]
    hkv, sk = A_k_cache.shape[1], A_k_cache.shape[2]
    assert A_x.shape == (1, 1, d) and HQ == 2 * hkv
    window = min(4096, max(256, sk // 4))
    copies, steps = _plan_program(_plan_units(d, ff, hkv, window))
    tail_start = ff - TAIL_COLS[-1]

    def kernel(x_hbm, k_hbm, v_hbm, wq_hbm, wo_hbm, w3_hbm, w4_hbm, gw_hbm, o_ref,
               x_buf, gw_buf, k_buf, v_buf, wq_buf, wo_buf, w3_buf, w4_buf,
               q_buf, attn_buf, tail_buf):
        refs = dict(k=(k_hbm, k_buf), v=(v_hbm, v_buf), wq=(wq_hbm, wq_buf),
                    wo=(wo_hbm, wo_buf), w3=(w3_hbm, w3_buf), w4=(w4_hbm, w4_buf))
        live = {}

        def down(hidden, acc, keep, r0, r1, c0, c1):
            w = w4_buf[pl.ds(r0, r1 - r0), pl.ds(c0, c1 - c0)]
            part = lax.dot_general(hidden, w, CONTRACT_LAST, preferred_element_type=F32)
            acc = acc + keep * part[0:1]
            if c1 == ff:
                o_ref[0, :, pl.ds(r0, r1 - r0)] = acc.astype(BF16)
            return acc

        def run(stage, *args):
            if stage == "pre":
                x = x_buf[0].astype(F32)
                gw = gw_buf[...].astype(F32).reshape(1, d)
                gate = jax.nn.sigmoid(jnp.sum(x * gw, axis=-1, keepdims=True))
                centered = x - jnp.mean(x, axis=-1, keepdims=True)
                var = jnp.mean(centered * centered, axis=-1, keepdims=True)
                live.update(x=x, gate=gate, keep=1.0 - gate,
                            normed=centered / jnp.sqrt(var + 1e-5))
            elif stage == "query":
                lhs = jnp.broadcast_to(live["x"], (ROWS, d)).astype(BF16)
                q = jnp.dot(lhs, wq_buf[...], preferred_element_type=F32)
                odd = lax.broadcasted_iota(jnp.int32, (ROWS, DH), 0) % 2 == 1
                for h in range(hkv):
                    c = 2 * DH * h
                    q_buf[h] = jnp.where(
                        odd, q[:, c + DH:c + 2 * DH], q[:, c:c + DH]).astype(BF16)
            elif stage == "hidden":
                lhs = jnp.broadcast_to(live["normed"], (ROWS, d)).astype(BF16)
                pre = jnp.dot(lhs, w3_buf[...], preferred_element_type=F32)
                live["hidden"] = jax.nn.gelu(pre, approximate=True).astype(BF16)
                tail_buf[...] = live["hidden"][:, tail_start:]
            elif stage == "head":
                (h,) = args
                s = lax.dot_general(q_buf[h], k_buf[h], CONTRACT_LAST,
                                    preferred_element_type=F32) * (DH ** -0.5)
                p = jnp.exp(s - jnp.max(s, axis=-1, keepdims=True))
                denom = jnp.sum(p, axis=-1, keepdims=True)
                attn_buf[h] = jnp.dot(p.astype(BF16), v_buf[h],
                                      preferred_element_type=F32) / denom
            elif stage == "project":
                cols = []
                for h in range(hkv):
                    o = attn_buf[h]
                    cols += [jnp.broadcast_to(o[i:i + 1], (ROWS, DH)) for i in range(2)]
                merged = jnp.concatenate(cols, axis=1).astype(BF16)
                attn = lax.dot_general(merged, wo_buf[...], CONTRACT_LAST,
                                       preferred_element_type=F32)[0:1]
                live["base"] = live["gate"] * attn + live["keep"] * live["x"]
            else:
                r0, r1, c0, c1 = args
                acc = live["base"][:, r0:r1] if c0 == 0 else live["acc"]
                live["acc"] = down(live["hidden"][:, c0:c1], acc, live["keep"], *args)

        def stream(sems):
            def descriptors(i):
                unit, piece, _ = copies[i]
                src, dst = refs[piece[0]]
                if piece[0] in ("k", "v"):
                    _, h, r = piece
                    src = src.at[0, h, pl.ds(sk - window + r, KV_PIECE_ROWS), :]
                    dst = dst.at[h, pl.ds(r, KV_PIECE_ROWS), :]
                else:
                    _, r, rows, c, cols = piece
                    src = src.at[pl.ds(r, rows), pl.ds(c, cols)]
                    dst = dst.at[pl.ds(r, rows), pl.ds(c, cols)]
                out = [pltpu.make_async_copy(src, dst, sems.at[unit % NUM_SEMS])]
                if i == 0:
                    out += [pltpu.make_async_copy(x_hbm, x_buf, sems.at[0]),
                            pltpu.make_async_copy(gw_hbm, gw_buf, sems.at[0])]
                return out

            for op, arg in steps[:-1]:
                if op == "run":
                    run(*arg)
                    continue
                for copy in descriptors(arg):
                    if op == "start":
                        copy.start(priority=copies[arg][2])
                    else:
                        copy.wait()
            return live["acc"], live["keep"]

        acc, keep = pl.run_scoped(stream, pltpu.SemaphoreType.DMA((NUM_SEMS,)))
        down(tail_buf[...], acc, keep, *steps[-1][1][1:])

    hbm = pl.BlockSpec(memory_space=pl.ANY)
    return pl.pallas_call(
        kernel,
        name="gated_mix_decode",
        out_shape=jax.ShapeDtypeStruct((1, 1, d), BF16),
        in_specs=[hbm] * 8,
        out_specs=pl.BlockSpec(memory_space=pltpu.VMEM),
        scratch_shapes=[
            pltpu.VMEM((1, 1, d), BF16),
            pltpu.VMEM((d,), BF16),
            pltpu.VMEM((hkv, window, DH), BF16),
            pltpu.VMEM((hkv, window, DH), BF16),
            pltpu.VMEM((d, HQ * DH), BF16),
            pltpu.VMEM((d, HQ * DH), BF16),
            pltpu.VMEM((d, ff), BF16),
            pltpu.VMEM((d, ff), BF16),
            pltpu.VMEM((hkv, ROWS, DH), BF16),
            pltpu.VMEM((hkv, ROWS, DH), F32),
            pltpu.VMEM((ROWS, TAIL_COLS[-1]), BF16),
        ],
        compiler_params=pltpu.CompilerParams(vmem_limit_bytes=80 * 1024 * 1024),
    )(A_x, A_k_cache, A_v_cache, A_wq, A_wo.T, B_w3, B_w4.T, gate_w)
```

```python
import jax
import jax.numpy as jnp
from jax import lax
from jax.experimental import pallas as pl
from jax.experimental.pallas import tpu as pltpu

F32, BF16 = jnp.float32, jnp.bfloat16
CONTRACT_LAST = (((1,), (1,)), ((), ()))
HQ, DH = 32, 128
LANES = 128
ROWS = 8

KV_PIECE_ROWS = 128
WEIGHT_PIECE_ROWS = 8
HEADS_PER_UNIT = 4
TAIL_COLS = (2560, 1024, 1024)
IN_FLIGHT = 104
TICK = 32
LAG = 20


def _round_robin(streams):
    longest = max(len(s) for s in streams)
    return [s[i] for i in range(longest) for s in streams if i < len(s)]


def _streams(pieces, count):
    cuts = [len(pieces) * i // count for i in range(count + 1)]
    return [pieces[a:b] for a, b in zip(cuts[:-1], cuts[1:])]


def _blocks(name, r0, r1, c0, c1, rows, cols):
    return [(name, r, rows, c, cols)
            for r in range(r0, r1, rows) for c in range(c0, c1, cols)]


def _plan_units(d, ff, hkv, window):
    def weight(name, ncols, r0, r1):
        return _blocks(name, r0, r1, 0, ncols, WEIGHT_PIECE_ROWS, ncols // 2)

    units = [(
        _round_robin(_streams(weight("wq", HQ * DH, 0, d), 4)
                     + _streams(weight("w3", ff, 0, d), 4)),
        [("pre",), ("query",), ("hidden",)],
    )]
    for first in range(0, hkv, HEADS_PER_UNIT):
        heads = range(first, first + HEADS_PER_UNIT)
        units.append((
            _round_robin([[(t, h, r) for r in range(0, window, KV_PIECE_ROWS)]
                          for h in heads for t in ("k", "v")]),
            [("head", h) for h in heads],
        ))
    units.append((_round_robin(_streams(weight("wo", HQ * DH, 0, d), 8)), [("project",)]))

    whole = d // LANES * LANES
    last = whole - LANES
    for row_ranges in (((whole, d), (0, last - LANES)), ((last - LANES, last),)):
        pieces = [p for r0, r1 in row_ranges for p in weight("w4", ff, r0, r1)]
        stages = [("down", r, min(r + LANES, r1), 0, ff)
                  for r0, r1 in row_ranges for r in range(r0, r1, LANES)]
        units.append((_round_robin(_streams(pieces, 4)), stages))
    c0 = 0
    for cols in TAIL_COLS:
        rows, width = (WEIGHT_PIECE_ROWS, cols // 2) if cols > 2048 else (16384 // cols, cols)
        pieces = _blocks("w4", last, whole, c0, c0 + cols, rows, width)
        units.append((_round_robin(_streams(pieces, 4)), [("down", last, whole, c0, c0 + cols)]))
        c0 += cols
    assert c0 == ff
    return units


def _plan_program(units):
    pieces = [(u, p) for u, (ps, _) in enumerate(units) for p in ps]
    n = len(pieces)
    lag = LAG + (n - LAG) % 2
    copies = [(u, p, i % 2 if i < n - lag else 1) for i, (u, p) in enumerate(pieces)]
    queues = [[i for i in range(n) if copies[i][2] == q] for q in (0, 1)]
    pairs = zip(queues[0], queues[1][lag:])
    order = queues[1][:lag] + [i for pair in pairs for i in pair]
    assert sorted(order) == list(range(n))

    steps, ready = [], []
    started = waited = end = 0

    def top_up():
        nonlocal started
        target = min(waited + IN_FLIGHT, n)
        steps.extend(("start", i) for i in order[started:target])
        started = target

    top_up()
    for ps, stages in units:
        end += len(ps)
        while waited < end:
            stop = end if end - waited < TICK * 3 // 2 else waited + TICK
            assert set(order[:started]).issuperset(range(waited, stop))
            steps += [("wait", i) for i in range(waited, stop)]
            waited = stop
            if waited == end:
                ready += stages
            top_up()
            count = len(ready) if started == n else 1
            steps += [("run", s) for s in ready[:count]]
            ready = ready[count:]
    assert not ready
    return copies, steps


@jax.jit
def pallas_gated_mix__sliding_block_cached__mixer_s_mlp__decode_kernel(
    A_x: jax.Array,
    A_k_cache: jax.Array,
    A_v_cache: jax.Array,
    A_wq: jax.Array,
    A_wo: jax.Array,
    B_x: jax.Array,
    B_w1: jax.Array,
    B_w2: jax.Array,
    B_w3: jax.Array,
    B_w4: jax.Array,
    gate_w: jax.Array,
):
    del B_x, B_w1, B_w2
    d = A_x.shape[-1]
    ff = B_w3.shape[-1]
    hkv, sk = A_k_cache.shape[1], A_k_cache.shape[2]
    assert A_x.shape == (1, 1, d) and HQ == 2 * hkv
    window = min(4096, max(256, sk // 4))
    units = _plan_units(d, ff, hkv, window)
    copies, steps = _plan_program(units)

    def kernel(x_hbm, k_hbm, v_hbm, wq_hbm, wo_hbm, w3_hbm, w4_hbm, gw_hbm, o_ref,
               x_buf, gw_buf, k_buf, v_buf, wq_buf, wo_buf, w3_buf, w4_buf,
               q_buf, attn_buf):
        refs = dict(k=(k_hbm, k_buf), v=(v_hbm, v_buf), wq=(wq_hbm, wq_buf),
                    wo=(wo_hbm, wo_buf), w3=(w3_hbm, w3_buf), w4=(w4_hbm, w4_buf))
        live = {}

        def run(stage, *args):
            if stage == "pre":
                x = x_buf[0].astype(F32)
                gw = gw_buf[...].astype(F32).reshape(1, d)
                gate = jax.nn.sigmoid(jnp.sum(x * gw, axis=-1, keepdims=True))
                centered = x - jnp.mean(x, axis=-1, keepdims=True)
                var = jnp.mean(centered * centered, axis=-1, keepdims=True)
                live.update(x=x, gate=gate, keep=1.0 - gate,
                            normed=centered / jnp.sqrt(var + 1e-5))
            elif stage == "query":
                lhs = jnp.broadcast_to(live["x"], (ROWS, d)).astype(BF16)
                q = jnp.dot(lhs, wq_buf[...], preferred_element_type=F32)
                odd = lax.broadcasted_iota(jnp.int32, (ROWS, DH), 0) % 2 == 1
                for h in range(hkv):
                    c = 2 * DH * h
                    q_buf[h] = jnp.where(
                        odd, q[:, c + DH:c + 2 * DH], q[:, c:c + DH]).astype(BF16)
            elif stage == "hidden":
                lhs = jnp.broadcast_to(live["normed"], (ROWS, d)).astype(BF16)
                pre = jnp.dot(lhs, w3_buf[...], preferred_element_type=F32)
                live["hidden"] = jax.nn.gelu(pre, approximate=True).astype(BF16)
            elif stage == "head":
                (h,) = args
                s = lax.dot_general(q_buf[h], k_buf[h], CONTRACT_LAST,
                                    preferred_element_type=F32) * (DH ** -0.5)
                p = jnp.exp(s - jnp.max(s, axis=-1, keepdims=True))
                denom = jnp.sum(p, axis=-1, keepdims=True)
                attn_buf[h] = jnp.dot(p.astype(BF16), v_buf[h],
                                      preferred_element_type=F32) / denom
            elif stage == "project":
                cols = []
                for h in range(hkv):
                    o = attn_buf[h]
                    cols += [jnp.broadcast_to(o[i:i + 1], (ROWS, DH)) for i in range(2)]
                merged = jnp.concatenate(cols, axis=1).astype(BF16)
                attn = lax.dot_general(merged, wo_buf[...], CONTRACT_LAST,
                                       preferred_element_type=F32)[0:1]
                live["base"] = live["gate"] * attn + live["keep"] * live["x"]
            else:
                r0, r1, c0, c1 = args
                part = lax.dot_general(
                    live["hidden"][:, c0:c1],
                    w4_buf[pl.ds(r0, r1 - r0), pl.ds(c0, c1 - c0)],
                    CONTRACT_LAST, preferred_element_type=F32)[0:1]
                acc = live["base"][:, r0:r1] if c0 == 0 else live["acc"]
                live["acc"] = acc + live["keep"] * part
                if c1 == ff:
                    o_ref[0, :, pl.ds(r0, r1 - r0)] = live["acc"].astype(BF16)

        def stream(sems):
            def descriptors(i):
                unit, piece, _ = copies[i]
                src, dst = refs[piece[0]]
                if piece[0] in ("k", "v"):
                    _, h, r = piece
                    src = src.at[0, h, pl.ds(sk - window + r, KV_PIECE_ROWS), :]
                    dst = dst.at[h, pl.ds(r, KV_PIECE_ROWS), :]
                else:
                    _, r, rows, c, cols = piece
                    src = src.at[pl.ds(r, rows), pl.ds(c, cols)]
                    dst = dst.at[pl.ds(r, rows), pl.ds(c, cols)]
                out = [pltpu.make_async_copy(src, dst, sems.at[unit])]
                if i == 0:
                    out += [pltpu.make_async_copy(x_hbm, x_buf, sems.at[0]),
                            pltpu.make_async_copy(gw_hbm, gw_buf, sems.at[0])]
                return out

            for op, arg in steps:
                if op == "run":
                    run(*arg)
                    continue
                for copy in descriptors(arg):
                    if op == "start":
                        copy.start(priority=copies[arg][2])
                    else:
                        copy.wait()

        pl.run_scoped(stream, pltpu.SemaphoreType.DMA((len(units),)))

    hbm = pl.BlockSpec(memory_space=pl.ANY)
    return pl.pallas_call(
        kernel,
        name="gated_mix_decode",
        out_shape=jax.ShapeDtypeStruct((1, 1, d), BF16),
        in_specs=[hbm] * 8,
        out_specs=pl.BlockSpec(memory_space=pltpu.VMEM),
        scratch_shapes=[
            pltpu.VMEM((1, 1, d), BF16),
            pltpu.VMEM((d,), BF16),
            pltpu.VMEM((hkv, window, DH), BF16),
            pltpu.VMEM((hkv, window, DH), BF16),
            pltpu.VMEM((d, HQ * DH), BF16),
            pltpu.VMEM((d, HQ * DH), BF16),
            pltpu.VMEM((d, ff), BF16),
            pltpu.VMEM((d, ff), BF16),
            pltpu.VMEM((hkv, ROWS, DH), BF16),
            pltpu.VMEM((hkv, ROWS, DH), F32),
        ],
        compiler_params=pltpu.CompilerParams(vmem_limit_bytes=80 * 1024 * 1024),
    )(A_x, A_k_cache, A_v_cache, A_wq, A_wo.T, B_w3, B_w4.T, gate_w)
```
